```python
import os as _os
_os.environ.setdefault("JAX_PLATFORMS", "cpu")
import jax
import jax.numpy as jnp

def _softmax(x, axis=-1):
    return jax.nn.softmax(x, axis=axis)
def _gelu(x):
    return jax.nn.gelu(x, approximate=True)
def _silu(x):
    return jax.nn.silu(x)
def _sigmoid(x):
    return jax.nn.sigmoid(x)
def _layernorm(x, axis=-1, eps=1e-5):
    m = jnp.mean(x, axis=axis, keepdims=True)
    v = jnp.var(x, axis=axis, keepdims=True)
    return (x - m) / jnp.sqrt(v + eps)
def _scatter_add(tgt, idx, src, axis=0):
    return tgt.at[idx].add(src)
def _segment_sum(src, seg, n):
    return jax.ops.segment_sum(src, seg, n)
class _Rng:
    def __init__(self, key):
        self._k = key
    def _next(self):
        self._k, sub = jax.random.split(self._k)
        return sub
    def normal(self, shape):
        return jax.random.normal(self._next(), shape, dtype=jnp.bfloat16)
    def randint(self, lo, hi, shape):
        return jax.random.randint(self._next(), shape, lo, hi, dtype=jnp.int32)
    def uniform(self, shape, lo=0.0, hi=1.0):
        return jax.random.uniform(self._next(), shape, jnp.bfloat16, lo, hi)
    def permutation(self, n):
        return jax.random.permutation(self._next(), n)


kernel_name = 'interleave_layers__linear_kernel_hedgehog__dense_activation_silu__prompt'

def setup_inputs():
    _rng = _Rng(jax.random.key(int.from_bytes(__import__("os").urandom(4), "little")))
    _w = (lambda a: (lambda t: t.astype(jnp.bfloat16) if jnp.issubdtype(t.dtype, jnp.floating) else t)(jnp.asarray(a)))
    def _A_setup():
        B, S, D, H = 1, 2048, 640, 32
        Dh = D // H
        return {
            "x": _w((lambda *s: _rng.normal(s) * 0.05)(B, S, D)),
            "wqkv": _w((lambda *s: _rng.normal(s) * 0.4)(D, 3 * D)),
            "w_phi": _w((lambda *s: _rng.normal(s) * 0.4)(H, Dh, Dh) * (Dh ** -0.5)),
            "wo": _w((lambda *s: _rng.normal(s) * 0.05)(D, D)),
        }
    _A_in = _A_setup()

    def _B_setup():
        B, S, D, F = 1, 2048, 640, 1728
        return {
            "x": _w((lambda *s: _rng.normal(s) * 0.05)(B, S, D)),
            "w1": _w((lambda *s: _rng.normal(s) * 1.6)(D, F) * (D ** -0.5)),
            "w2": _w((lambda *s: _rng.normal(s) * 1.6)(F, D) * (F ** -0.5)),
        }
    _B_in = _B_setup()

    return {
        "A_x": _A_in["x"],
        "A_wqkv": _A_in["wqkv"],
        "A_w_phi": _A_in["w_phi"],
        "A_wo": _A_in["wo"],
        "B_x": _B_in["x"],
        "B_w1": _B_in["w1"],
        "B_w2": _B_in["w2"],
    }

def reference(A_x, A_wqkv, A_w_phi, A_wo, B_x, B_w1, B_w2):
    def _A_ref(x, wqkv, w_phi, wo):
        B, S, D = x.shape
        H = 32; Dh = D // H
        qkv = (lambda x, *d: x.transpose(*d))((x @ wqkv).reshape(B, S, 3, H, Dh), 2, 0, 3, 1, 4)
        q, k, v = qkv[0], qkv[1], qkv[2]
        pq = jnp.einsum("bhsd,hdf->bhsf", q, w_phi)
        pk = jnp.einsum("bhsd,hdf->bhsf", k, w_phi)
        phi_q = jnp.concatenate([_softmax(pq, axis=-1), _softmax(-pq, axis=-1)], axis=-1)
        phi_k = jnp.concatenate([_softmax(pk, axis=-1), _softmax(-pk, axis=-1)], axis=-1)
        kv = jnp.einsum("bhsf,bhsd->bhfd", phi_k, v)
        z  = jnp.einsum("bhsf->bhf", phi_k)
        num = jnp.einsum("bhqf,bhfd->bhqd", phi_q, kv)
        den = jnp.einsum("bhqf,bhf->bhq", phi_q, z)[..., None] + 1e-6
        o = num / den
        return (lambda x, *d: x.transpose(*d))(o, 0, 2, 1, 3).reshape(B, S, D) @ wo

    def _B_ref(x, w1, w2):
        h = jnp.einsum("bsd,df->bsf", x, w1)
        h = _silu(h)
        out = jnp.einsum("bsf,fd->bsd", h, w2)
        return out

    x = A_x
    x = x + _A_ref(_layernorm(x, axis=-1), A_wqkv, A_w_phi, A_wo)
    x = x + _B_ref(_layernorm(x, axis=-1), B_w1, B_w2)
    x = x + _A_ref(_layernorm(x, axis=-1), A_wqkv, A_w_phi, A_wo)
    x = x + _B_ref(_layernorm(x, axis=-1), B_w1, B_w2)
    return x
```

```python
import functools
import jax
import jax.numpy as jnp
from jax import lax
import jax.experimental.pallas as pl
import jax.experimental.pallas.tpu as pltpu

S, D, H, DH, F = 2048, 640, 32, 20, 1728
NG = 8
TM = 512
NB = S // TM
BF = jnp.bfloat16
F32 = jnp.float32


def _idiv(x, n):
    return jnp.floor((x.astype(F32) + 0.5) * (1.0 / n)).astype(jnp.int32)


def _layernorm_t(xt):
    m = jnp.sum(xt, axis=0, keepdims=True) * (1.0 / D)
    xc = xt - m
    v = jnp.sum(xc * xc, axis=0, keepdims=True) * (1.0 / D)
    return xc * lax.rsqrt(v + 1e-5)


def _nt(a, b):
    return lax.dot_general(a, b, (((1,), (1,)), ((), ())), preferred_element_type=F32)


def _nn(a, b):
    return jnp.dot(a, b, preferred_element_type=F32)


def _dual_softmax(L):
    T = L.shape[-1]
    ng = L.shape[0] // 80
    L4 = L.reshape(ng, 10, 8, T)
    mx = jnp.max(L4, axis=1)
    mn = jnp.min(L4, axis=1)
    mx = jnp.maximum(mx, pltpu.roll(mx, 4, 1))
    mn = jnp.minimum(mn, pltpu.roll(mn, 4, 1))
    ep = jnp.exp(L4 - mx[:, None])
    en = jnp.exp(mn[:, None] - L4)
    sp = jnp.sum(ep, axis=1)
    sn = jnp.sum(en, axis=1)
    sp = sp + pltpu.roll(sp, 4, 1)
    sn = sn + pltpu.roll(sn, 4, 1)
    pp = ep * (1.0 / sp)[:, None]
    pn = en * (1.0 / sn)[:, None]
    phi = jnp.concatenate([pp, pn], axis=1)
    return phi.reshape(ng * 160, T)


_KT_GROUPS = [((128 * k) // 20 // 4, (128 * k + 127) // 20 // 4) for k in range(5)]
_FT_GROUPS = [((128 * n) // 160, (128 * n + 127) // 160) for n in range(10)]


def _sparse_perm_dot(a, w, nt):
    parts = []
    for k, (glo, ghi) in enumerate(_KT_GROUPS):
        ak = a[80 * glo:80 * (ghi + 1), 128 * k:128 * (k + 1)]
        if nt:
            parts.append(_nt(ak, w[:, 128 * k:128 * (k + 1)]))
        else:
            parts.append(_nn(ak, w[128 * k:128 * (k + 1), :]))
    rows = []
    for g in range(NG):
        acc = None
        for k, (glo, ghi) in enumerate(_KT_GROUPS):
            if glo <= g <= ghi:
                p = parts[k][80 * (g - glo):80 * (g - glo + 1)]
                acc = p if acc is None else acc + p
        rows.append(acc)
    return jnp.concatenate(rows, axis=0)


def _kernel(x_hbm, wqkv_hbm, wphi_ref, wo_hbm, w1t_hbm, w2_hbm, out_hbm,
            xin_ref, wqkv_ref, wo_ref, w1t_ref, w2_ref,
            xt_ref, xn_ref, wt_ref, wot_ref, w2t_ref, phiq_ref, kvt_ref, zacc_ref, kvz_ref,
            wsem, qsem, xsem, osem):
    def wcopy(i):
        src, dst = ((wo_hbm, wo_ref), (w1t_hbm, w1t_ref), (w2_hbm, w2_ref))[i]
        return pltpu.make_async_copy(src, dst, wsem.at[i])

    def qcopy(n):
        rows = pl.ds(128 * n, 128)
        return pltpu.make_async_copy(wqkv_hbm.at[rows, :], wqkv_ref.at[rows, :], qsem.at[n])

    def xcopy(b):
        rows = pl.ds(b * TM, TM)
        return pltpu.make_async_copy(x_hbm.at[rows, :], xin_ref.at[rows, :], xsem.at[b])

    def ocopy(b):
        rows = pl.ds(b * TM, TM)
        return pltpu.make_async_copy(xin_ref.at[rows, :], out_hbm.at[rows, :], osem.at[b])

    def prep_block(b):
        cols = pl.ds(pl.multiple_of(b * TM, TM), TM)
        xt = xin_ref[cols, :].astype(F32).T
        xt_ref[:, cols] = xt
        xn_ref[...] = _layernorm_t(xt).astype(BF)

    qcopy(0).start()
    qcopy(1).start()

    r = lax.broadcasted_iota(jnp.int32, (D, 1), 0)
    c = lax.broadcasted_iota(jnp.int32, (1, D), 1)
    g_r = _idiv(r, 80)
    rem = r - 80 * g_r
    fd_r = rem >> 2
    h_r = 4 * g_r + (rem & 3)
    h_c = _idiv(c, 20)
    same_head = h_r == h_c
    e = jnp.where(fd_r == lax.broadcasted_iota(jnp.int32, (1, DH), 1), 1.0, 0.0).astype(BF)
    a_full = _nt(e, wphi_ref[...])
    a_qk = jnp.where(same_head, a_full, 0.0).astype(BF)

    for n in range(5):
        qcopy(n).wait()
        if n + 2 < 5:
            qcopy(n + 2).start()
        elif n + 2 == 5:
            xcopy(0).start()
        else:
            xcopy(1).start()
        rows = slice(128 * n, 128 * (n + 1))
        wt_ref[0:D, rows] = _sparse_perm_dot(a_qk, wqkv_ref[rows, 0:D], True).astype(BF)
        wt_ref[D:2 * D, rows] = _sparse_perm_dot(a_qk, wqkv_ref[rows, D:2 * D], True).astype(BF)
        wt_ref[2 * D:3 * D, rows] = wqkv_ref[rows, 2 * D:3 * D].T
    xcopy(0).wait()
    for b in range(2, NB):
        xcopy(b).start()
    prep_block(0)
    for i in range(3):
        wcopy(i).start()

    hkv_r = _idiv(r, 20)
    cc = lax.broadcasted_iota(jnp.int32, (1, 2 * D), 1)
    gcc = _idiv(cc, 160)
    hkv_c = 4 * gcc + ((cc - 160 * gcc) & 3)
    zr = lax.broadcasted_iota(jnp.int32, (NG * 16, 1), 0)
    hz_r = 4 * (zr >> 4) + (zr & 3)

    def qkv_feat(xn, b):
        qkvt = _nn(wt_ref[...], xn)
        phi = _dual_softmax(qkvt[0:2 * D])
        phiq = phi[0:2 * D].astype(BF)
        phik_f = phi[2 * D:4 * D]
        phik = phik_f.astype(BF)
        vt = qkvt[2 * D:3 * D].astype(BF)
        phiq_ref[:, pl.ds(pl.multiple_of(b * TM, TM), TM)] = phiq
        zs = phik_f[:, 0:128]
        for t in range(1, TM // 128):
            zs = zs + phik_f[:, 128 * t:128 * (t + 1)]
        zacc_ref[...] += zs
        for n, (glo, ghi) in enumerate(_FT_GROUPS):
            r0, r1 = 80 * glo, 80 * (ghi + 1)
            kvt_ref[r0:r1, 128 * n:128 * (n + 1)] += _nt(vt[r0:r1], phik[128 * n:128 * (n + 1)])

    def zero_acc():
        zacc_ref[...] = jnp.zeros(zacc_ref.shape, F32)
        for n, (glo, ghi) in enumerate(_FT_GROUPS):
            r0, r1 = 80 * glo, 80 * (ghi + 1)
            kvt_ref[r0:r1, 128 * n:128 * (n + 1)] = jnp.zeros((r1 - r0, 128), F32)

    def finalize_kvz():
        zrow = jnp.sum(zacc_ref[...].T, axis=0, keepdims=True)
        for n, (glo, ghi) in enumerate(_FT_GROUPS):
            hc = hkv_c[:, 128 * n:128 * (n + 1)]
            for g in range(glo, ghi + 1):
                blk = kvt_ref[80 * g:80 * g + 80, 128 * n:128 * (n + 1)]
                kvz_ref[96 * g:96 * g + 80, 128 * n:128 * (n + 1)] = (
                    jnp.where(hkv_r[80 * g:80 * g + 80] == hc, blk, 0.0).astype(BF))
                kvz_ref[96 * g + 80:96 * g + 96, 128 * n:128 * (n + 1)] = (
                    jnp.where(hz_r[16 * g:16 * g + 16] == hc, zrow[:, 128 * n:128 * (n + 1)], 0.0).astype(BF))

    def attn_ffn(xt, b):
        phiq = phiq_ref[:, pl.ds(pl.multiple_of(b * TM, TM), TM)]
        parts = []
        for i, (glo, ghi) in enumerate(_FT_GROUPS):
            parts.append(_nn(kvz_ref[96 * glo:96 * (ghi + 1), 128 * i:128 * (i + 1)],
                             phiq[128 * i:128 * (i + 1)]))
        os_ = []
        for g in range(NG):
            a = (160 * g) // 128
            off_a = 96 * (g - (128 * a) // 160)
            off_b = 96 * (g - (128 * (a + 1)) // 160)
            nd = parts[a][off_a:off_a + 96] + parts[a + 1][off_b:off_b + 96]
            num = nd[0:80].reshape(10, 8, TM)
            rden = 1.0 / (nd[80:88] + 1e-6)
            bj = [jnp.broadcast_to(rden[j:j + 1, :], (8, TM)) for j in range(4)]
            low = lax.broadcasted_iota(jnp.int32, (8, TM), 0) < 4
            mult = jnp.stack([bj[0], bj[0], jnp.where(low, bj[0], bj[1]), bj[1], bj[1],
                              bj[2], bj[2], jnp.where(low, bj[2], bj[3]), bj[3], bj[3]], axis=0)
            os_.append((num * mult).reshape(80, TM))
        ot = jnp.concatenate(os_, axis=0).astype(BF)
        x1 = xt + _nn(wot_ref[...], ot)
        xn = _layernorm_t(x1).astype(BF)
        hh = _nn(w1t_ref[...], xn)
        hh = hh * jax.nn.sigmoid(hh)
        x2 = x1 + _nn(w2t_ref[...], hh.astype(BF))
        return x2

    def layer(l, carry):
        zero_acc()

        @pl.when(l == 1)
        def _():
            prep_block(0)

        def pa(b, c):
            @pl.when(jnp.logical_and(l == 0, b + 1 < NB))
            def _():
                xcopy(b + 1).wait()
            qkv_feat(xn_ref[...], b)
            prep_block(jnp.minimum(b + 1, NB - 1))
            return c
        with jax.named_scope('PA'):
            lax.fori_loop(0, NB, pa, 0)
        finalize_kvz()

        @pl.when(l == 0)
        def _():
            wcopy(0).wait()
            wcopy(1).wait()
            wcopy(2).wait()
            wot_ref[...] = wo_ref[...].T
            w2t_ref[...] = w2_ref[...].T

        def pb(b, c):
            cols = pl.ds(pl.multiple_of(b * TM, TM), TM)
            x2 = attn_ffn(xt_ref[:, cols], b)
            xin_ref[cols, :] = x2.astype(BF).T

            @pl.when(l == 1)
            def _():
                ocopy(b).start()
            return c
        with jax.named_scope('PB'):
            lax.fori_loop(0, NB, pb, 0)
        return carry
    lax.fori_loop(0, 2, layer, 0)

    for b in range(NB):
        ocopy(b).wait()


@jax.jit
def pallas_interleave_layers__linear_kernel_hedgehog__dense_activation_silu__prompt_kernel(A_x, A_wqkv, A_w_phi, A_wo, B_x, B_w1, B_w2):
    x = A_x.reshape(S, D)
    wphi = A_w_phi.reshape(H * DH, DH)
    w1t = B_w1.T
    any_spec = pl.BlockSpec(memory_space=pl.ANY)
    out = pl.pallas_call(
        _kernel,
        out_shape=jax.ShapeDtypeStruct((S, D), BF),
        in_specs=[any_spec, any_spec, pl.BlockSpec(memory_space=pltpu.VMEM), any_spec, any_spec, any_spec],
        out_specs=any_spec,
        scratch_shapes=[
            pltpu.VMEM((S, D), BF),
            pltpu.VMEM((D, 3 * D), BF),
            pltpu.VMEM((D, D), BF),
            pltpu.VMEM((F, D), BF),
            pltpu.VMEM((F, D), BF),
            pltpu.VMEM((D, S), F32),
            pltpu.VMEM((D, TM), BF),
            pltpu.VMEM((3 * D, D), BF),
            pltpu.VMEM((D, D), BF),
            pltpu.VMEM((D, F), BF),
            pltpu.VMEM((2 * D, S), BF),
            pltpu.VMEM((D, 2 * D), F32),
            pltpu.VMEM((2 * D, 128), F32),
            pltpu.VMEM((NG * 96, 2 * D), BF),
            pltpu.SemaphoreType.DMA((3,)),
            pltpu.SemaphoreType.DMA((5,)),
            pltpu.SemaphoreType.DMA((NB,)),
            pltpu.SemaphoreType.DMA((NB,)),
        ],
        compiler_params=pltpu.CompilerParams(vmem_limit_bytes=110 * 1024 * 1024),
    )(x, A_wqkv, wphi, A_wo, w1t, B_w2)
    return out.reshape(1, S, D)
```

```python
import jax
import jax.numpy as jnp
from jax import lax
import jax.experimental.pallas as pl
import jax.experimental.pallas.tpu as pltpu

S, D, H, DH, F = 2048, 640, 32, 20, 1728
NG = 8
TM = 512
NB = S // TM
BF = jnp.bfloat16
F32 = jnp.float32


def _idiv(x, n):
    return jnp.floor((x.astype(F32) + 0.5) * (1.0 / n)).astype(jnp.int32)


def _layernorm_t(xt):
    m = jnp.sum(xt, axis=0, keepdims=True) * (1.0 / D)
    xc = xt - m
    v = jnp.sum(xc * xc, axis=0, keepdims=True) * (1.0 / D)
    return xc * lax.rsqrt(v + 1e-5)


def _nt(a, b):
    return lax.dot_general(a, b, (((1,), (1,)), ((), ())), preferred_element_type=F32)


def _nn(a, b):
    return jnp.dot(a, b, preferred_element_type=F32)


def _dual_softmax(L):
    T = L.shape[-1]
    ng = L.shape[0] // 80
    L4 = L.reshape(ng, 10, 8, T)
    mx = jnp.max(L4, axis=1)
    mn = jnp.min(L4, axis=1)
    mx = jnp.maximum(mx, pltpu.roll(mx, 4, 1))
    mn = jnp.minimum(mn, pltpu.roll(mn, 4, 1))
    ep = jnp.exp(L4 - mx[:, None])
    en = jnp.exp(mn[:, None] - L4)
    sp = jnp.sum(ep, axis=1)
    sn = jnp.sum(en, axis=1)
    sp = sp + pltpu.roll(sp, 4, 1)
    sn = sn + pltpu.roll(sn, 4, 1)
    pp = ep * (1.0 / sp)[:, None]
    pn = en * (1.0 / sn)[:, None]
    phi = jnp.concatenate([pp, pn], axis=1)
    return phi.reshape(ng * 160, T)


_KT_GROUPS = [((128 * k) // 20 // 4, (128 * k + 127) // 20 // 4) for k in range(5)]
_FT_GROUPS = [((128 * n) // 160, (128 * n + 127) // 160) for n in range(10)]


def _sparse_fold(a, w):
    parts = []
    for k, (glo, ghi) in enumerate(_KT_GROUPS):
        parts.append(_nt(a[80 * glo:80 * (ghi + 1), 128 * k:128 * (k + 1)], w[:, 128 * k:128 * (k + 1)]))
    rows = []
    for g in range(NG):
        acc = None
        for k, (glo, ghi) in enumerate(_KT_GROUPS):
            if glo <= g <= ghi:
                p = parts[k][80 * (g - glo):80 * (g - glo + 1)]
                acc = p if acc is None else acc + p
        rows.append(acc)
    return jnp.concatenate(rows, axis=0)


def _kernel(x_hbm, wqkv_hbm, wphi_ref, wo_hbm, w1t_hbm, w2_hbm, out_hbm,
            xin_ref, wqkv_ref, wo_ref, w1t_ref, w2_ref,
            xn_ref, wt_ref, wot_ref, w2t_ref, phiq_ref, kvt_ref, zacc_ref, kvz_ref,
            wsem, qsem, xsem, osem):
    def wcopy(i):
        src, dst = ((wo_hbm, wo_ref), (w1t_hbm, w1t_ref), (w2_hbm, w2_ref))[i]
        return pltpu.make_async_copy(src, dst, wsem.at[i])

    def qcopy(n):
        rows = pl.ds(128 * n, 128)
        return pltpu.make_async_copy(wqkv_hbm.at[rows, :], wqkv_ref.at[rows, :], qsem.at[n])

    def xcopy(b):
        rows = pl.ds(b * TM, TM)
        return pltpu.make_async_copy(x_hbm.at[rows, :], xin_ref.at[rows, :], xsem.at[b])

    def ocopy(b):
        rows = pl.ds(b * TM, TM)
        return pltpu.make_async_copy(xin_ref.at[rows, :], out_hbm.at[rows, :], osem.at[b])

    def prep_block(b):
        cols = pl.ds(pl.multiple_of(b * TM, TM), TM)
        xt = xin_ref[cols, :].astype(F32).T
        xn_ref[...] = _layernorm_t(xt).astype(BF)

    qcopy(0).start()
    qcopy(1).start()

    r = lax.broadcasted_iota(jnp.int32, (D, 1), 0)
    c = lax.broadcasted_iota(jnp.int32, (1, D), 1)
    g_r = _idiv(r, 80)
    rem = r - 80 * g_r
    f_r = rem >> 2
    h_r = 4 * g_r + (rem & 3)
    h_c = _idiv(c, 20)
    e = jnp.where(f_r == lax.broadcasted_iota(jnp.int32, (1, DH), 1), 1.0, 0.0).astype(BF)
    a_full = _nt(e, wphi_ref[...])
    a_qk = jnp.where(h_r == h_c, a_full, 0.0).astype(BF)

    def fold_chunk(n):
        rows = slice(128 * n, 128 * (n + 1))
        wt_ref[0:D, rows] = _sparse_fold(a_qk, wqkv_ref[rows, 0:D]).astype(BF)
        wt_ref[D:2 * D, rows] = _sparse_fold(a_qk, wqkv_ref[rows, D:2 * D]).astype(BF)
        wt_ref[2 * D:3 * D, rows] = wqkv_ref[rows, 2 * D:3 * D].T

    qcopy(0).wait()
    xcopy(0).start()
    fold_chunk(0)
    qcopy(1).wait()
    qcopy(2).start()
    fold_chunk(1)
    xcopy(0).wait()
    qcopy(3).start()
    prep_block(0)
    qcopy(2).wait()
    qcopy(4).start()
    fold_chunk(2)
    qcopy(3).wait()
    xcopy(1).start()
    fold_chunk(3)
    qcopy(4).wait()
    for b in range(2, NB):
        xcopy(b).start()
    for i in range(3):
        wcopy(i).start()
    fold_chunk(4)

    hkv_r = _idiv(r, 20)
    cc = lax.broadcasted_iota(jnp.int32, (1, 2 * D), 1)
    gcc = _idiv(cc, 160)
    hkv_c = 4 * gcc + ((cc - 160 * gcc) & 3)
    zr = lax.broadcasted_iota(jnp.int32, (NG * 16, 1), 0)
    hz_r = 4 * (zr >> 4) + (zr & 3)

    def qkv_feat(xn, b):
        qkvt = _nn(wt_ref[...], xn)
        phi = _dual_softmax(qkvt[0:2 * D])
        phiq = phi[0:2 * D].astype(BF)
        phik_f = phi[2 * D:4 * D]
        phik = phik_f.astype(BF)
        vt = qkvt[2 * D:3 * D].astype(BF)
        phiq_ref[:, pl.ds(pl.multiple_of(b * TM, TM), TM)] = phiq
        zs = phik_f[:, 0:128]
        for t in range(1, TM // 128):
            zs = zs + phik_f[:, 128 * t:128 * (t + 1)]
        zacc_ref[...] += zs
        for n, (glo, ghi) in enumerate(_FT_GROUPS):
            r0, r1 = 80 * glo, 80 * (ghi + 1)
            kvt_ref[r0:r1, 128 * n:128 * (n + 1)] += _nt(vt[r0:r1], phik[128 * n:128 * (n + 1)])

    def zero_acc():
        zacc_ref[...] = jnp.zeros(zacc_ref.shape, F32)
        for n, (glo, ghi) in enumerate(_FT_GROUPS):
            r0, r1 = 80 * glo, 80 * (ghi + 1)
            kvt_ref[r0:r1, 128 * n:128 * (n + 1)] = jnp.zeros((r1 - r0, 128), F32)

    def finalize_kvz():
        zrow = jnp.sum(zacc_ref[...].T, axis=0, keepdims=True)
        for n, (glo, ghi) in enumerate(_FT_GROUPS):
            hc = hkv_c[:, 128 * n:128 * (n + 1)]
            for g in range(glo, ghi + 1):
                blk = kvt_ref[80 * g:80 * g + 80, 128 * n:128 * (n + 1)]
                kvz_ref[96 * g:96 * g + 80, 128 * n:128 * (n + 1)] = (
                    jnp.where(hkv_r[80 * g:80 * g + 80] == hc, blk, 0.0).astype(BF))
                kvz_ref[96 * g + 80:96 * g + 96, 128 * n:128 * (n + 1)] = (
                    jnp.where(hz_r[16 * g:16 * g + 16] == hc, zrow[:, 128 * n:128 * (n + 1)], 0.0).astype(BF))

    def attn_ffn(xt, b):
        phiq = phiq_ref[:, pl.ds(pl.multiple_of(b * TM, TM), TM)]
        parts = []
        for i, (glo, ghi) in enumerate(_FT_GROUPS):
            parts.append(_nn(kvz_ref[96 * glo:96 * (ghi + 1), 128 * i:128 * (i + 1)],
                             phiq[128 * i:128 * (i + 1)]))
        low = lax.broadcasted_iota(jnp.int32, (8, TM), 0) < 4
        os_ = []
        for g in range(NG):
            a = (160 * g) // 128
            off_a = 96 * (g - (128 * a) // 160)
            off_b = 96 * (g - (128 * (a + 1)) // 160)
            nd = parts[a][off_a:off_a + 96] + parts[a + 1][off_b:off_b + 96]
            num = nd[0:80].reshape(10, 8, TM)
            rden = 1.0 / (nd[80:88] + 1e-6)
            bj = [jnp.broadcast_to(rden[j:j + 1, :], (8, TM)) for j in range(4)]
            mult = jnp.stack([bj[0], bj[0], jnp.where(low, bj[0], bj[1]), bj[1], bj[1],
                              bj[2], bj[2], jnp.where(low, bj[2], bj[3]), bj[3], bj[3]], axis=0)
            os_.append((num * mult).reshape(80, TM))
        ot = jnp.concatenate(os_, axis=0).astype(BF)
        x1 = xt + _nn(wot_ref[...], ot)
        xn = _layernorm_t(x1).astype(BF)
        hh = _nn(w1t_ref[...], xn)
        hh = hh * jax.nn.sigmoid(hh)
        return x1 + _nn(w2t_ref[...], hh.astype(BF))

    def layer(l, carry):
        zero_acc()

        @pl.when(l == 1)
        def _():
            prep_block(0)

        def pa(b, c):
            @pl.when(jnp.logical_and(l == 0, b + 1 < NB))
            def _():
                xcopy(b + 1).wait()
            qkv_feat(xn_ref[...], b)
            prep_block(jnp.minimum(b + 1, NB - 1))
            return c
        lax.fori_loop(0, NB, pa, 0)

        @pl.when(l == 0)
        def _():
            wcopy(0).wait()
            wcopy(1).wait()
            wcopy(2).wait()
            finalize_kvz()
            wot_ref[...] = wo_ref[...].T
            w2t_ref[...] = w2_ref[...].T

        @pl.when(l == 1)
        def _():
            finalize_kvz()

        def pb(b, c):
            cols = pl.ds(pl.multiple_of(b * TM, TM), TM)
            x2 = attn_ffn(xin_ref[cols, :].astype(F32).T, b)
            xin_ref[cols, :] = x2.astype(BF).T

            @pl.when(l == 1)
            def _():
                ocopy(b).start()
            return c
        lax.fori_loop(0, NB, pb, 0)
        return carry
    lax.fori_loop(0, 2, layer, 0)

    for b in range(NB):
        ocopy(b).wait()


@jax.jit
def pallas_interleave_layers__linear_kernel_hedgehog__dense_activation_silu__prompt_kernel(
    A_x: jax.Array,
    A_wqkv: jax.Array,
    A_w_phi: jax.Array,
    A_wo: jax.Array,
    B_x: jax.Array,
    B_w1: jax.Array,
    B_w2: jax.Array,
):
    x = A_x.reshape(S, D)
    wphi = A_w_phi.reshape(H * DH, DH)
    w1t = B_w1.T
    any_spec = pl.BlockSpec(memory_space=pl.ANY)
    out = pl.pallas_call(
        _kernel,
        out_shape=jax.ShapeDtypeStruct((S, D), BF),
        in_specs=[any_spec, any_spec, pl.BlockSpec(memory_space=pltpu.VMEM), any_spec, any_spec, any_spec],
        out_specs=any_spec,
        scratch_shapes=[
            pltpu.VMEM((S, D), BF),
            pltpu.VMEM((D, 3 * D), BF),
            pltpu.VMEM((D, D), BF),
            pltpu.VMEM((F, D), BF),
            pltpu.VMEM((F, D), BF),
            pltpu.VMEM((D, TM), BF),
            pltpu.VMEM((3 * D, D), BF),
            pltpu.VMEM((D, D), BF),
            pltpu.VMEM((D, F), BF),
            pltpu.VMEM((2 * D, S), BF),
            pltpu.VMEM((D, 2 * D), F32),
            pltpu.VMEM((2 * D, 128), F32),
            pltpu.VMEM((NG * 96, 2 * D), BF),
            pltpu.SemaphoreType.DMA((3,)),
            pltpu.SemaphoreType.DMA((5,)),
            pltpu.SemaphoreType.DMA((NB,)),
            pltpu.SemaphoreType.DMA((NB,)),
        ],
        compiler_params=pltpu.CompilerParams(vmem_limit_bytes=100 * 1024 * 1024),
    )(x, A_wqkv, wphi, A_wo, w1t, B_w2)
    return out.reshape(1, S, D)
```
